```python
import os as _os
_os.environ.setdefault('JAX_PLATFORMS', 'cpu')
import jax
import jax.numpy as jnp

def _softmax(x, axis=-1):
    return jax.nn.softmax(x, axis=axis)

def _gelu(x):
    return jax.nn.gelu(x, approximate=True)

def _silu(x):
    return jax.nn.silu(x)

def _sigmoid(x):
    return jax.nn.sigmoid(x)

def _layernorm(x, axis=-1, eps=1e-05):
    m = jnp.mean(x, axis=axis, keepdims=True)
    v = jnp.var(x, axis=axis, keepdims=True)
    return (x - m) / jnp.sqrt(v + eps)

def _scatter_add(tgt, idx, src, axis=0):
    return tgt.at[idx].add(src)

def _segment_sum(src, seg, n):
    return jax.ops.segment_sum(src, seg, n)

class _Rng:

    def __init__(self, key):
        self._k = key

    def _next(self):
        self._k, sub = jax.random.split(self._k)
        return sub

    def normal(self, shape):
        return jax.random.normal(self._next(), shape, dtype=jnp.bfloat16)

    def randint(self, lo, hi, shape):
        return jax.random.randint(self._next(), shape, lo, hi, dtype=jnp.int32)

    def uniform(self, shape, lo=0.0, hi=1.0):
        return jax.random.uniform(self._next(), shape, jnp.bfloat16, lo, hi)

    def permutation(self, n):
        return jax.random.permutation(self._next(), n)
kernel_name = 'adaLN_cond__grouped_kv_mqa__swiglu_ffn__prompt'

def setup_inputs():
    _rng = _Rng(jax.random.key(int.from_bytes(__import__("os").urandom(4), "little")))
    _w = lambda a: (lambda t: t.astype(jnp.bfloat16) if jnp.issubdtype(t.dtype, jnp.floating) else t)(jnp.asarray(a))

    def _A_setup():
        B, S, D, H = (1, 2048, 576, 32)
        Dh = D // H
        return {'x': _w((lambda *s: _rng.normal(s) * 0.05)(B, S, D)), 'wq': _w((lambda *s: _rng.normal(s) * 0.05)(D, H * Dh)), 'wk': _w((lambda *s: _rng.normal(s) * 0.05)(D, Dh)), 'wv': _w((lambda *s: _rng.normal(s) * 0.05)(D, Dh)), 'wo': _w((lambda *s: _rng.normal(s) * 0.05)(H * Dh, D))}
    _A_in = _A_setup()

    def _B_setup():
        B, S, D, F = (1, 2048, 576, 4608)
        return {'x': _w((lambda *s: _rng.normal(s) * 0.05)(B, S, D)), 'w_gate': _w((lambda *s: _rng.normal(s) * 0.05)(D, F)), 'w_up': _w((lambda *s: _rng.normal(s) * 0.05)(D, F)), 'w_down': _w((lambda *s: _rng.normal(s) * 0.05)(F, D))}
    _B_in = _B_setup()
    return {'A_x': _A_in['x'], 'A_wq': _A_in['wq'], 'A_wk': _A_in['wk'], 'A_wv': _A_in['wv'], 'A_wo': _A_in['wo'], 'B_x': _B_in['x'], 'B_w_gate': _B_in['w_gate'], 'B_w_up': _B_in['w_up'], 'B_w_down': _B_in['w_down'], 'c': _w((lambda *s: _rng.normal(s) * 0.05)(1, 576) * 8.0), 'w_mod': _w((lambda *s: _rng.normal(s) * 0.05)(576, 6 * 576) * 576 ** (-0.5) * 8.0)}

def reference(A_x, A_wq, A_wk, A_wv, A_wo, B_x, B_w_gate, B_w_up, B_w_down, c, w_mod):

    def _A_ref(x, wq, wk, wv, wo):
        B, S, D = x.shape
        H = 32
        Dh = D // H
        q = (lambda x, *d: x.transpose(*d))((x @ wq).reshape(B, S, H, Dh), 0, 2, 1, 3)
        k = x @ wk
        v = x @ wv
        scores = jnp.einsum('bhqd,bkd->bhqk', q, k) * Dh ** (-0.5)
        p = _softmax(scores, axis=-1)
        o = jnp.einsum('bhqk,bkd->bhqd', p, v)
        return (lambda x, *d: x.transpose(*d))(o, 0, 2, 1, 3).reshape(B, S, H * Dh) @ wo

    def _B_ref(x, w_gate, w_up, w_down):
        g = _silu(x @ w_gate)
        u = x @ w_up
        return g * u @ w_down
    x = A_x
    mod = (_silu(c) @ w_mod).reshape(c.shape[0], 6, 1, -1)
    sa, ca, ga, sb, cb, gb = (mod[:, 0].copy(), mod[:, 1].copy(), mod[:, 2].copy(), mod[:, 3].copy(), mod[:, 4].copy(), mod[:, 5].copy())
    h = _layernorm(x, axis=-1) * (1 + ca) + sa
    x = x + ga * _A_ref(h, A_wq, A_wk, A_wv, A_wo)
    h = _layernorm(x, axis=-1) * (1 + cb) + sb
    x = x + gb * _B_ref(h, B_w_gate, B_w_up, B_w_down)
    return x
```

```python
import functools
import math

import jax
import jax.numpy as jnp
from jax import lax
import jax.experimental.pallas as pl
import jax.experimental.pallas.tpu as pltpu

S, D, H, DH, F = 2048, 576, 32, 18, 4608
LANES = 128
NT = S // LANES
EPS = 1e-5
KV = 24
QKV = D + 2 * KV
BF16, F32 = jnp.bfloat16, jnp.float32
NT_DIMS = (((1,), (1,)), ((), ()))
L_MIN, L_MAX, O_MAX = 2.0 ** -60, 2.0 ** 100, 3.0e38


def _ln_mod(x, scale1, shift):
    mean = jnp.sum(x, axis=0, keepdims=True) * (1.0 / D)
    d = x - mean
    var = jnp.sum(d * d, axis=0, keepdims=True) * (1.0 / D)
    return d * lax.rsqrt(var + EPS) * scale1 + shift


def _kernel(c_ref, wkT_ref, wvT_ref, xT_hbm, wq_hbm, wo_hbm, wg_hbm, wu_hbm, wdT_hbm, wmod_hbm,
            out_hbm,
            x_v, wq_v, wo_v, wg_v, wu_v, wdT_v, wmod_v,
            modc, wqkvT, woT, q_s, k_s, v_s, o_s, bad_s, x1_s, h2_s, acc_s, out_v, sems,
            *, TB, FC, LAG):
    NB = S // TB
    TPB = TB // LANES

    def copy(src, dst, i):
        return pltpu.make_async_copy(src, dst, sems.at[i])

    cp_mod_a = copy(wmod_hbm.at[:, pl.ds(0, 2 * D)], wmod_v.at[:, pl.ds(0, 2 * D)], 0)
    cp_wq = copy(wq_hbm, wq_v, 1)
    cp_mod_b = copy(wmod_hbm.at[:, pl.ds(2 * D, 4 * D)], wmod_v.at[:, pl.ds(2 * D, 4 * D)], 2)
    cp_wo = copy(wo_hbm, wo_v, 3)
    cp_wg = copy(wg_hbm, wg_v, 4)
    cp_wu = copy(wu_hbm, wu_v, 5)
    cp_wd = copy(wdT_hbm, wdT_v, 6)
    cp_x = [copy(xT_hbm.at[:, pl.ds(b * TB, TB)], x_v.at[b], 7 + b) for b in range(NB)]

    cp_wq.start()
    cp_mod_a.start()
    for cp in cp_x:
        cp.start()

    cf = c_ref[...].astype(F32)
    sc = jnp.broadcast_to(cf * jax.nn.sigmoid(cf), (16, D)).astype(BF16)

    def mod_columns(lo, n):
        m = jnp.dot(sc, wmod_v[:, lo:lo + n], preferred_element_type=F32)
        modc[lo:lo + n, :] = jnp.broadcast_to(m[0:1, :], (LANES, n)).T

    pad = jnp.zeros((KV - DH, D), F32)
    wqkvT[D:QKV, :] = jnp.concatenate(
        [wkT_ref[...].astype(F32), pad, wvT_ref[...].astype(F32), pad], axis=0).astype(BF16)
    cp_wq.wait()
    wqkvT[0:D, :] = wq_v[...].astype(F32).T.astype(BF16)
    cp_mod_a.wait()
    mod_columns(0, 2 * D)

    kscale = DH ** -0.5 * math.log2(math.e)
    for b in range(NB):
        cp_x[b].wait()
        if b == NB - 1:
            for cp in (cp_mod_b, cp_wo, cp_wg, cp_wu, cp_wd):
                cp.start()
        hs = []
        for j in range(TPB):
            x = x_v[b, :, j * LANES:(j + 1) * LANES].astype(F32)
            hs.append(_ln_mod(x, 1.0 + modc[D:2 * D, :], modc[0:D, :]).astype(BF16))
        qkv = jnp.dot(wqkvT[...], jnp.concatenate(hs, axis=1), preferred_element_type=F32)
        for j in range(TPB):
            t = b * TPB + j
            blk = qkv[:, j * LANES:(j + 1) * LANES]
            q_s[t] = blk[0:D + 16]
            kt = blk[D:D + KV] * kscale
            kt = jnp.concatenate([kt, jnp.zeros((LANES - KV, LANES), F32)], axis=0)
            k_s[t * LANES:(t + 1) * LANES, :] = kt.T[:, 0:32].astype(BF16)
            vt = blk[D + KV:QKV].astype(BF16).astype(F32)
            row = lax.broadcasted_iota(jnp.int32, (KV, LANES), 0)
            v_s[:, t * LANES:(t + 1) * LANES] = jnp.where(row == DH, 1.0, vt)

    bad_s[...] = jnp.zeros(bad_s.shape, F32)

    def load_q(t, g):
        return jnp.concatenate(
            [q_s[t, pl.ds(DH * (4 * g + i), 32), :] for i in range(4)], axis=1).astype(BF16)

    def attn_tile(t, carry):
        items = [(g, kt) for g in range(H // 4) for kt in range(NT)]
        ps, accs, qs = {}, {}, {}
        bad = [bad_s[...]]

        def qk(g, kt):
            if kt == 0:
                qs[g] = load_q(t, g)
            s = jnp.dot(k_s[kt * LANES:(kt + 1) * LANES, :], qs[g], preferred_element_type=F32)
            ps[(g, kt)] = jnp.exp2(s).astype(BF16)

        def pv(g, kt):
            o = jnp.dot(v_s[:, kt * LANES:(kt + 1) * LANES], ps.pop((g, kt)),
                        preferred_element_type=F32)
            accs[g] = o if kt == 0 else accs[g] + o
            if kt == NT - 1:
                a = accs.pop(g)
                l = a[DH:DH + 1, :]
                ok = (l >= L_MIN) & (l <= L_MAX) & (jnp.abs(a) <= O_MAX)
                bad[0] = jnp.maximum(bad[0], jnp.where(ok, 0.0, 1.0))
                a = a * (1.0 / l)
                for i in range(4):
                    o_s[t, pl.ds(DH * (4 * g + i), KV), :] = a[:, i * LANES:(i + 1) * LANES]

        for n in range(len(items) + LAG):
            if n < len(items):
                qk(*items[n])
            if n >= LAG:
                pv(*items[n - LAG])
        bad_s[...] = bad[0]
        return carry

    lax.fori_loop(0, NT, attn_tile, 0)

    @pl.when(jnp.max(bad_s[...]) > 0.0)
    def _():
        def safe_tile(n, carry):
            t, g = n // (H // 4), n % (H // 4)
            base = pl.multiple_of(g * 4 * DH, 8)
            qg = q_s[t, pl.ds(base, 4 * DH + 16), :]
            q = jnp.concatenate([qg[DH * i:DH * i + 32] for i in range(4)], axis=1).astype(BF16)
            s = jnp.dot(k_s[...], q, preferred_element_type=F32)
            p = jnp.exp2(s - jnp.max(s, axis=0, keepdims=True)).astype(BF16)
            a = jnp.dot(v_s[...], p, preferred_element_type=F32)
            a = a * (1.0 / a[DH:DH + 1, :])
            o_s[t, pl.ds(base, 4 * DH), :] = jnp.concatenate(
                [a[0:DH, i * LANES:(i + 1) * LANES] for i in range(4)], axis=0)
            return carry
        lax.fori_loop(0, NT * (H // 4), safe_tile, 0)

    cp_mod_b.wait()
    mod_columns(2 * D, 4 * D)
    cp_wo.wait()
    woT[...] = wo_v[...].astype(F32).T.astype(BF16)
    cp_wg.wait()
    cp_wu.wait()
    cp_wd.wait()

    def out_copy(b):
        return pltpu.make_async_copy(
            out_v.at[b], out_hbm.at[:, pl.ds(pl.multiple_of(b * TB, TB), TB)], sems.at[7 + b])

    def ffn_block(b, carry):
        o = jnp.concatenate([o_s[b * TPB + j, 0:D, :] for j in range(TPB)], axis=1).astype(BF16)
        attn = jnp.dot(woT[...], o, preferred_element_type=F32)
        for j in range(TPB):
            sl = slice(j * LANES, (j + 1) * LANES)
            x1 = x_v[b, :, sl].astype(F32) + modc[2 * D:3 * D, :] * attn[:, sl]
            x1_s[:, sl] = x1
            h = _ln_mod(x1, 1.0 + modc[4 * D:5 * D, :], modc[3 * D:4 * D, :])
            h2_s[sl, :] = h.T.astype(BF16)
        acc_s[...] = jnp.zeros(acc_s.shape, F32)

        def chunk(f, carry2):
            col = pl.ds(pl.multiple_of(f * FC, LANES), FC)
            h2 = h2_s[...]
            g = jnp.dot(h2, wg_v[:, col], preferred_element_type=F32)
            u = jnp.dot(h2, wu_v[:, col], preferred_element_type=F32)
            a = (g * jax.nn.sigmoid(g) * u).astype(BF16)
            acc_s[...] += lax.dot_general(wdT_v[:, col], a, NT_DIMS, preferred_element_type=F32)
            return carry2

        lax.fori_loop(0, F // FC, chunk, 0)
        for j in range(TPB):
            sl = slice(j * LANES, (j + 1) * LANES)
            out_v[b, :, sl] = (x1_s[:, sl] + modc[5 * D:6 * D, :] * acc_s[:, sl]).astype(BF16)
        out_copy(b).start()
        return carry

    lax.fori_loop(0, NB, ffn_block, 0)
    for b in range(NB):
        out_copy(b).wait()


def make(TB=512, FC=1536, LAG=2):
    NB = S // TB

    def fn(A_x, A_wq, A_wk, A_wv, A_wo, B_x, B_w_gate, B_w_up, B_w_down, c, w_mod):
        del B_x
        vmem = pl.BlockSpec(memory_space=pltpu.VMEM)
        hbm = pl.BlockSpec(memory_space=pl.ANY)
        outT = pl.pallas_call(
            functools.partial(_kernel, TB=TB, FC=FC, LAG=LAG),
            out_shape=jax.ShapeDtypeStruct((D, S), BF16),
            in_specs=[vmem, vmem, vmem] + [hbm] * 7,
            out_specs=hbm,
            scratch_shapes=[
                pltpu.VMEM((NB, D, TB), BF16),
                pltpu.VMEM((D, D), BF16),
                pltpu.VMEM((D, D), BF16),
                pltpu.VMEM((D, F), BF16),
                pltpu.VMEM((D, F), BF16),
                pltpu.VMEM((D, F), BF16),
                pltpu.VMEM((D, 6 * D), BF16),
                pltpu.VMEM((6 * D, LANES), F32),
                pltpu.VMEM((QKV, D), BF16),
                pltpu.VMEM((D, D), BF16),
                pltpu.VMEM((NT, D + 16, LANES), F32),
                pltpu.VMEM((S, 32), BF16),
                pltpu.VMEM((KV, S), F32),
                pltpu.VMEM((NT, D + 8, LANES), F32),
                pltpu.VMEM((KV, 4 * LANES), F32),
                pltpu.VMEM((D, TB), F32),
                pltpu.VMEM((TB, D), BF16),
                pltpu.VMEM((D, TB), F32),
                pltpu.VMEM((NB, D, TB), BF16),
                pltpu.SemaphoreType.DMA((7 + NB,)),
            ],
            compiler_params=pltpu.CompilerParams(vmem_limit_bytes=110 * 2 ** 20),
            name="adaln_mqa_swiglu",
        )(c, A_wk.T, A_wv.T, A_x.reshape(S, D).T, A_wq, A_wo, B_w_gate, B_w_up, B_w_down.T, w_mod)
        return outT.T.reshape(1, S, D)

    return jax.jit(fn)


_kernel_fn = make()


@jax.jit
def pallas_adaLN_cond__grouped_kv_mqa__swiglu_ffn__prompt_kernel(
    A_x, A_wq, A_wk, A_wv, A_wo, B_x, B_w_gate, B_w_up, B_w_down, c, w_mod,
):
    return _kernel_fn(A_x, A_wq, A_wk, A_wv, A_wo, B_x, B_w_gate, B_w_up, B_w_down, c, w_mod)
```

```python
import functools
import math

import jax
import jax.numpy as jnp
from jax import lax
import jax.experimental.pallas as pl
import jax.experimental.pallas.tpu as pltpu

S, D, H, DH, F = 2048, 576, 32, 18, 4608
LANES = 128
NT = S // LANES
TB = 4 * LANES
NB = S // TB
QD, QF = D // 4, F // 4
NU = QF // LANES
EPS = 1e-5
KV = 24
NMXU = 4
BF16, F32, U32 = jnp.bfloat16, jnp.float32, jnp.uint32
NT_DIMS = (((1,), (1,)), ((), ()))
L_MIN, L_MAX, V_MAX = 2.0 ** -60, 2.0 ** 100, 2.0 ** 20

VPOS = ((0, 5, 10), (1, 6, 11), (3, 8, 13), (4, 9, 14))
NV = len(VPOS[0])


def _lhs7(a11, a12, a21, a22):
    return [a11 + a22, a21 + a22, a11, a22, a11 + a12, a21 - a11, a12 - a22]


def _rhs7(b11, b12, b21, b22, swap=False):
    if swap:
        b11, b12, b21, b22 = b12, b11, b22, b21
    return [b11 + b22, b11, b12 - b22, b21 - b11, b22, b11 + b12, b21 + b22]


def _out7(m, swap=False):
    c11, c12 = ((m[0] + m[3]) - m[4]) + m[6], m[2] + m[4]
    c21, c22 = m[1] + m[3], ((m[0] - m[1]) + m[2]) + m[5]
    return [c12, c11, c22, c21] if swap else [c11, c12, c21, c22]


KA, KB = 192, 64
DEPTH = (KA, KB, 256, 256, 256, 256, 256, 256, 128, 128)
PASS_DEPTH = [d // 2 if d > LANES else d for d in DEPTH for _ in range(7 if d > LANES else 2)]
POFF = [sum(7 if d > LANES else 2 for d in DEPTH[:p]) for p in range(len(DEPTH) + 1)]


def _gu_factors(a, b, c, sign):
    return [[a[0]], [b[0]], [a[1], sign(b[1])], [a[2], b[3]], [a[3], b[2]], [a[4], sign(b[4])],
            [a[5], c[1]], [a[6], c[0]], [b[5], c[2]], [b[6], c[3]]]


def _gu_lhs(h1, h2):
    cut = lambda h: (h[0:KA], h[KA:2 * KA], h[2 * KA:2 * KA + KB], h[2 * KA + KB:D - KB], h[D - KB:D])
    x, y = cut(h1), cut(h2)
    return _gu_factors(_lhs7(x[0], x[1], y[0], y[1]), _lhs7(x[2], x[3], y[2], y[3]),
                       (x[4], y[4], y[4], x[4]), lambda v: -v)


def _gu_out(p):
    return [((p[0] + p[4]) - p[5]) + p[7], ((p[5] + p[3]) + p[1]) + p[9],
            ((p[4] + p[2]) + p[1]) + p[8], ((p[0] - p[2]) + p[3]) + p[6]]


DOWN_SWAP = (False, False, True, False, True, True, True)


def _pack(x):
    return pltpu.bitcast(x, U32)


def _unpack(x):
    return pltpu.bitcast(x, BF16)


def _dot(a, b):
    return jnp.dot(a, b, preferred_element_type=F32)


def _ln_mod(x, scale, shift):
    d = x - jnp.sum(x, axis=0, keepdims=True) * (1.0 / D)
    var = jnp.sum(d * d, axis=0, keepdims=True) * (1.0 / D)
    return d * lax.rsqrt(var + EPS) * scale + shift


class _Spread:
    def __init__(self, jobs, slots, zero_s):
        self.jobs, self.rate = list(jobs), sum(job[1] for job in jobs) / slots
        self.zero, self.credit = pl.multiple_of(zero_s[0], 16), 0.0

    def under(self, results):
        for m in range(0, results[0].shape[0], 8):
            self.credit += self.rate
            while self.jobs and self.credit > 0:
                src, cost, fn = self.jobs.pop(0)
                self.credit -= cost
                mark = pltpu.bitcast(results[len(self.jobs) % len(results)][m:m + 8], src.dtype)
                src[pl.ds(self.zero + src.shape[0] - 16, mark.shape[0]), 0:LANES] = mark
                fn()


import os


def scoped(name, fn):
    if not os.environ.get("SCOPES"):
        return fn

    def run(*a):
        with jax.named_scope(name):
            return fn(*a)
    return run


def _kernel(c_hbm, wkT_hbm, wvT_hbm, xT_hbm, wq_hbm, wo_hbm, wg_hbm, wu_hbm, wdT_hbm, wmod_hbm,
            out_hbm,
            c_ref, wkT_ref, wvT_ref, x_v, wq_v, wo_v, wg_v, wu_v, wdT_v, wmod_v,
            modc, wT, woT, q_s, k_s, kb_s, v_s, o_s, l_s, p_s, h2_s, wgu_s, wd_s, part0, part1, part2, zero_s, sems,
            *, NACC, HA, LEAD, SKIP, BDT, UP, WO, DROP, UNR):
    parts = (part0, part1, part2)

    def copy(src, dst, i):
        return pltpu.make_async_copy(src, dst, sems.at[i])

    cuts = (0, 5 * LANES, 2 * D, 6 * D)
    cp_mod = [copy(wmod_hbm.at[:, lo:hi], wmod_v.at[:, lo:hi], i) for i, (lo, hi) in enumerate(zip(cuts, cuts[1:]))]
    cp_wq = copy(wq_hbm, wq_v, 3)
    cp_small = [copy(src, dst, 12 + i) for i, (src, dst) in enumerate(((c_hbm, c_ref), (wkT_hbm, wkT_ref), (wvT_hbm, wvT_ref)))]
    cp_late = [cp_mod[2], copy(wo_hbm, wo_v, 4), copy(wg_hbm, wg_v.at[0:D], 5), copy(wu_hbm, wu_v.at[0:D], 6),
               copy(wdT_hbm, wdT_v.at[0:D], 7)]
    cp_x = [copy(xT_hbm.at[:, pl.ds(b * TB, TB)], x_v.at[b], 8 + b) for b in range(NB)]

    def out_copy(b):
        return copy(x_v.at[b], out_hbm.at[:, pl.ds(pl.multiple_of(b * TB, TB), TB)], 8 + b)

    for cp in cp_small + [cp_wq] + cp_mod[:2] + cp_x:
        cp.start()
    zero_s[0] = 0

    q_s[:, D:D + 16, :] = jnp.zeros((NT, 16, LANES), F32)
    p_s[...] = jnp.ones(p_s.shape, F32)
    for cp in cp_small:
        scoped('w_small', cp.wait)()
    cf = c_ref[...].astype(F32)
    sc = jnp.broadcast_to(cf * jax.nn.sigmoid(cf), (16, D)).astype(BF16)

    mod_scale, mod_shift = (1.0, 1.0, 1.0, 0.5, 0.5, 2.0), (0.0, 1.0, 0.0, 0.0, 0.5, 0.0)

    def mod_columns(part):
        lo, n = cuts[part], cuts[part + 1] - cuts[part]
        col = lax.broadcasted_iota(jnp.int32, (1, n), 1) + lo
        m = _dot(sc, wmod_v[:, lo:lo + n])[0:1, :]
        for i in range(lo // D, -(-(lo + n) // D)):
            m = jnp.where((col >= i * D) & (col < (i + 1) * D), m * mod_scale[i] + mod_shift[i], m)
        modc[lo:lo + n, :] = jnp.broadcast_to(m, (LANES, n)).T

    pad = jnp.zeros((KV - DH, D), F32)
    wT[0:KV, :] = _pack(jnp.concatenate(
        [wkT_ref[...].astype(F32), pad, wvT_ref[...].astype(F32), pad], axis=0).astype(BF16))
    scoped('w_wq', cp_wq.wait)()
    wT[KV:KV + D // 2, :] = _pack(wq_v[...].T)
    for i in range(2):
        scoped('w_mod', cp_mod[i].wait)()
        mod_columns(i)

    kscale = DH ** -0.5 * math.log2(math.e)

    def qkv(b):
        hs = [_ln_mod(x_v[b, :, j * LANES:(j + 1) * LANES].astype(F32), modc[D:2 * D, :], modc[0:D, :])
              for j in range(4)]
        h = jnp.concatenate(hs, axis=1).astype(BF16)
        res = _dot(_unpack(wT[...]), h)
        for j in range(4):
            t = 4 * b + j
            blk = res[:, j * LANES:(j + 1) * LANES]
            q_s[t, 0:D, :] = blk[2 * KV:]
            kk = jnp.concatenate([blk[0:KV] * kscale, jnp.zeros((LANES - KV, LANES), F32)], axis=0).T
            groups = [kk[8 * (15 - g):8 * (16 - g)] for g in range(16)]
            k_s[t] = jnp.concatenate(
                [groups[g] for g in range(16) if g not in VPOS[j]] + [groups[g] for g in VPOS[j]], axis=0)
            for r, g in enumerate(VPOS[j]):
                kb_s[t * NV + r] = jnp.concatenate(
                    [jnp.broadcast_to(groups[g][:, d:d + 1], (8, LANES)) for d in range(DH)], axis=0)
            row = lax.broadcasted_iota(jnp.int32, (KV, LANES), 0)
            v_s[:, t * LANES:(t + 1) * LANES] = jnp.where(row == DH, 1.0, blk[KV:2 * KV])

    scoped('w_x', cp_x[0].wait)()
    qkv(0)
    for cp in cp_x[1:]:
        scoped('w_late', cp.wait)()
    qkv(1)
    qkv(2)
    qkv(3)

    def weight_jobs(u):
        cols = [pl.ds(pl.multiple_of(j * QF + u * LANES, LANES), LANES) for j in range(4)]
        slots, jobs = {}, []

        def outer(w_v, where, combine, part_s, keys):
            raw = [_pack(w_v[pl.ds(r, 16), cols[j]]) for r, j in where]
            new = combine(*[jnp.concatenate([pltpu.unpack_elementwise(
                x, index=n, packed_dtype=BF16, unpacked_dtype=F32) for n in range(2)], axis=0) for x in raw])
            for key, v in zip(keys, new):
                part_s[pl.ds(16 * slots[key], 16), :] = v

        def inner(part_s, keys, combine, dst):
            for i, v in enumerate(combine(*[part_s[pl.ds(16 * slots[key], 16), :] for key in keys])):
                dst(i, pltpu.bitcast(pltpu.pack_elementwise([v[0:8], v[8:16]], packed_dtype=BF16), U32))

        def put_gu(n, k, r, i, v):
            wgu_s[u, k + i, pl.ds(r // 2, 8), n * LANES:(n + 1) * LANES] = v

        def put_down(p, r, i, v):
            wd_s[u, 7 * p + i, pl.ds(r // 2, 8), :] = v

        for n, w_v in enumerate((wg_v, wu_v)):
            used = 0
            for kind, (lo, size) in enumerate(((0, KA), (2 * KA, KB), (D - KB, KB))):
                for r in range(0, size, 16):
                    for j2 in range(2):
                        keys = [(n, kind, i, r, j2) for i in range(7 if kind < 2 else 2)]
                        slots.update((key, used + i) for i, key in enumerate(keys))
                        used += len(keys)
                        where = [(lo + k * size + r, 2 * j1 + j2) for k in range(2 if kind < 2 else 1) for j1 in range(2)]
                        combine = functools.partial(_rhs7, swap=kind == 1) if kind < 2 else lambda *w: w
                        jobs.append((w_v, WO if kind < 2 else 8, functools.partial(outer, w_v, where, combine, parts[n], keys)))
            index = _gu_factors(*[[(kind, i % 2 if kind == 2 else i) for i in range(7)] for kind in range(3)],
                                lambda v: v)
            for p, depth in enumerate(DEPTH):
                first = KA if index[p][0][0] == 0 else KB
                for r in range(0, PASS_DEPTH[POFF[p]], 16):
                    rows = (r, depth // 2 + r) if depth > LANES else (r,)
                    keys = [(n, *index[p][k >= first], k - first * (k >= first), j2) for k in rows for j2 in range(2)]
                    jobs.append((parts[n], 17 if depth > LANES else 6, functools.partial(
                        inner, parts[n], keys, _rhs7 if depth > LANES else lambda *w: w,
                        functools.partial(put_gu, n, POFF[p], r))))
        for r in range(0, QD, 16):
            for q in range(4):
                keys = [(2, p, r, q) for p in range(7)]
                slots.update((key, (r // 4 + q) * 7 + p) for p, key in enumerate(keys))
                where = [((2 * i1 + q // 2) * QD + r, 2 * j1 + q % 2) for i1 in range(2) for j1 in range(2)]
                jobs.append((wdT_v, WO, functools.partial(outer, wdT_v, where, _lhs7, parts[2], keys)))
        for r in range(0, QD, 16):
            for p in range(7):
                jobs.append((parts[2], 17, functools.partial(
                    inner, parts[2], [(2, p, r, q) for q in range(4)], _lhs7, functools.partial(put_down, p, r))))
        return jobs

    NC = NT // NMXU

    def values(slot, h, c, ps, acc):
        o = [_dot(v_s[:, pl.ds((NMXU * c + j) * LANES, LANES)], p) for j, p in enumerate(ps)]
        o = (o[0] + o[1]) + (o[2] + o[3])
        acc = acc + o if c else o
        if c == NC - 1:
            l = acc[DH:DH + 1, :]
            l_s[slot, h:h + 1, :] = l
            r = pltpu.reciprocal(l, approx=True)
            o_s[slot, pl.ds(DH * h, KV), :] = acc * (r * (2.0 - l * r))
        return acc

    def carried(slot):
        return slot, H - 1, NC - 1, [p_s[j] for j in range(NMXU)], p_s[NMXU, 0:KV, :]

    def attention(t, jobs):
        side = _Spread(jobs, UP * (16 - NV + 1), zero_s)
        qs, qb = {}, {}

        def scores(h, c):
            if c == 0:
                qh = q_s[t, pl.ds(DH * h, 32), :]
                qs[h] = qh.astype(BF16)
                rows = [jnp.broadcast_to(qh[d:d + 1], (8, LANES)) for d in range(DH)]
                qb[h] = [jnp.concatenate(rows[d:d + NACC], axis=0) for d in range(0, DH, NACC)]
            raw, ps = [], []
            nv = NV - bool(side.jobs)
            for j in range(NMXU):
                kt = NMXU * c + j
                if nv == NV:
                    k = k_s[kt, 0:LANES - 8 * NV, 0:32]
                else:
                    cut = 8 * (VPOS[j][DROP] - DROP)
                    k = [k_s[kt, pl.ds(LANES - 8 * (NV - DROP), 8), 0:32], k_s[kt, cut:LANES - 8 * NV, 0:32]]
                    k = jnp.concatenate([k_s[kt, 0:cut, 0:32]] + k if cut else k, axis=0)
                raw.append(_dot(k, qs[h]))
                p = jnp.exp2(raw[-1])
                blocks = [p[m:m + 8] for m in range(0, LANES - 8 * nv, 8)]
                for r, g in enumerate(VPOS[j]):
                    if nv < NV and r == DROP:
                        continue
                    part = None
                    for i, q in enumerate(qb[h]):
                        term = kb_s[kt * NV + r, pl.ds(i * NACC * 8, NACC * 8), :] * q
                        part = term if part is None else part + term
                    blocks.insert(g, jnp.exp2(sum((part[8 * i:8 * i + 8] for i in range(1, NACC)), part[0:8])))
                ps.append(jnp.concatenate(blocks[::-1], axis=0))
            side.under(raw)
            return ps

        todo = carried(t)
        for h in range(HA):
            for c in range(NC):
                ps = scores(h, c)
                todo = (t + 1, h, c, ps, values(*todo))
        for j in range(NMXU):
            p_s[j] = todo[3][j]
        p_s[NMXU, 0:KV, :] = todo[4]

    @pl.loop(0, NT - NU)
    def _(t):
        @pl.when(t == 1)
        def _():
            for cp in cp_late:
                cp.start()

        scoped("att", attention)(t, [])

    for cp in cp_late:
        cp.wait()
    pl.loop(0, NU)(scoped("attp", lambda u: attention(NT - NU + u, weight_jobs(u))))

    values(*carried(NT))
    woT[...] = _pack(wo_v[...].T)
    mod_columns(2)

    sums = l_s[1:NT + 1]
    bad = jnp.maximum(jnp.max(jnp.where((sums >= L_MIN) & (sums <= L_MAX), 0.0, 1.0)),
                      jnp.max(jnp.where(jnp.abs(v_s[...]) <= V_MAX, 0.0, 1.0)))

    @pl.when(bad > 0.0)
    def _():
        def safe(n, carry):
            t, g = n // (H // 4), n % (H // 4)
            base = pl.multiple_of(g * 4 * DH, 8)
            qg = q_s[t, pl.ds(base, 4 * DH + 16), :]
            q = jnp.concatenate([qg[DH * i:DH * i + 32] for i in range(4)], axis=1).astype(BF16)
            keys = []
            for kt in range(NT):
                order = [g for g in range(16) if g not in VPOS[kt % NMXU]] + list(VPOS[kt % NMXU])
                keys += [k_s[kt, pl.ds(8 * order.index(g), 8), 0:32] for g in range(15, -1, -1)]
            s = _dot(jnp.concatenate(keys, axis=0), q)
            a = _dot(v_s[...], jnp.exp2(s - jnp.max(s, axis=0, keepdims=True)).astype(BF16))
            a = a * (1.0 / a[DH:DH + 1, :])
            o_s[t + 1, pl.ds(base, 4 * DH), :] = jnp.concatenate(
                [a[0:DH, i * LANES:(i + 1) * LANES] for i in range(4)], axis=0)
            return carry
        lax.fori_loop(0, NT * (H // 4), safe, 0)

    def lhs_factors(b):
        hs = [_ln_mod(q_s[4 * b + j, 0:D, :], modc[4 * D:5 * D, :], modc[3 * D:4 * D, :]) for j in range(4)]
        outer = [_gu_lhs(hs[i2], hs[2 + i2]) for i2 in range(2)]
        for p, depth in enumerate(DEPTH):
            f = [jnp.concatenate(x[p], axis=0) for x in outer]
            if depth > LANES:
                f = _lhs7(*[x[k * depth // 2:(k + 1) * depth // 2] for x in f for k in range(2)])
            for i, v in enumerate(f):
                h2_s[POFF[p] + i, :, 0:v.shape[0]] = _pack(v.astype(BF16).T)

    for b in range(NB):
        o = jnp.concatenate([o_s[4 * b + j + 1, 0:D, :] for j in range(4)], axis=1).astype(BF16)
        attn = _dot(_unpack(woT[...]), o)
        for j in range(4):
            sl = slice(j * LANES, (j + 1) * LANES)
            q_s[4 * b + j, 0:D, :] = x_v[b, :, sl].astype(F32) + modc[2 * D:3 * D, :] * attn[:, sl]
        if b == 0:
            lhs_factors(0)

    def ffn_block(b, carry):
        def gate_up(u):
            def mm(kl, kr):
                return _dot(_unpack(h2_s[kl, :, 0:PASS_DEPTH[kl]]), _unpack(wgu_s[u, kr, 0:PASS_DEPTH[kr] // 2, :]))
            prod = {}
            for p in (0, 4, 5, 7, 2, 3, 6, 1, 8, 9):
                k = POFF[p]
                if DEPTH[p] > LANES:
                    m = {i: mm(k + i, k + i) for i in (0, 3, 1, 2, 4, 5, 6)}
                    prod[p] = _out7(m)
                else:
                    prod[p] = [mm(k + i2, k + j2) for i2 in range(2) for j2 in range(2)]
            act = {}
            for inner in range(4):
                for out, cc in enumerate(_gu_out([prod[p][inner] for p in range(10)])):
                    g, up = cc[:, :LANES], cc[:, LANES:]
                    act[out // 2, inner // 2, out % 2, inner % 2] = (g * jnp.tanh(g) + g) * up
            outer = [_rhs7(*[act[i1, i2, j1, j2] for j1 in range(2) for i1 in range(2)])
                     for j2 in range(2) for i2 in range(2)]
            return [v.astype(BDT) for p in range(7) for v in _rhs7(*[x[p] for x in outer], swap=DOWN_SWAP[p])]

        acts = [gate_up(u) for u in range(NU)]
        lhs_factors(jnp.minimum(b + 1, NB - 1))

        def down(pairs):
            return [lax.dot_general(_unpack(wd_s[u, p]), acts[u][p], NT_DIMS, preferred_element_type=F32)
                    for u, p in pairs]

        seq = [7 * p + i for p in (0, 3, 1, 2, 4, 5, 6) for i in (0, 3, 1, 2, 4, 5, 6)]
        m = {}
        for n in range(0, 49, 4):
            if n >= LEAD:
                for k in range(0 if n == LEAD else n, n + 1, 4):
                    for p, v in zip(seq[k:k + 4], down([(NU - 1, p) for p in seq[k:k + 4]])):
                        m[p] = m[p] + v if p in m else v
            for p in seq[n:n + 4]:
                for u0 in range(0, NU - 1, 4):
                    v = down([(u, p) for u in range(u0, u0 + 4)])
                    v = (v[0] + v[1]) + (v[2] + v[3])
                    m[p] = m[p] + v if p in m else v
        inner = [_out7([m[7 * p + i] for i in range(7)], swap=DOWN_SWAP[p]) for p in range(7)]
        y = [_out7([x[n] for x in inner]) for n in range(4)]
        for r1 in range(2):
            for r2 in range(2):
                rows = pl.ds((2 * r1 + r2) * QD, QD)
                g = modc[pl.ds(5 * D + rows.start, QD), :]
                x_v[b, rows, :] = jnp.concatenate(
                    [q_s[4 * b + 2 * i1 + i2, rows, :] + g * y[2 * r2 + i2][2 * r1 + i1]
                     for i1 in range(2) for i2 in range(2)], axis=1).astype(BF16)
        out_copy(b).start()
        return carry

    if 'f' not in SKIP:
        lax.fori_loop(0, NB, scoped('ffn', ffn_block), 0, unroll=UNR)
    for b in range(NB):
        scoped('w_out', out_copy(b).wait)()


def make(NACC=3, HA=32, LEAD=8, SKIP="", BDT="bf16", UP=50, WO=32, DROP=1, UNR=2):
    BDT = {"bf16": BF16, "f32": F32}[BDT]

    def fn(A_x, A_wq, A_wk, A_wv, A_wo, B_x, B_w_gate, B_w_up, B_w_down, c, w_mod):
        del B_x
        vmem = pl.BlockSpec(memory_space=pltpu.VMEM)
        hbm = pl.BlockSpec(memory_space=pl.ANY)
        outT = pl.pallas_call(
            functools.partial(_kernel, NACC=NACC, HA=HA, LEAD=LEAD, SKIP=SKIP, BDT=BDT, UP=UP, WO=WO, DROP=DROP, UNR=UNR),
            out_shape=jax.ShapeDtypeStruct((D, S), BF16),
            in_specs=[hbm] * 10,
            out_specs=hbm,
            scratch_shapes=[
                pltpu.VMEM((1, D), BF16),
                pltpu.VMEM((DH, D), BF16),
                pltpu.VMEM((DH, D), BF16),
                pltpu.VMEM((NB, D, TB), BF16),
                pltpu.VMEM((D, D), BF16),
                pltpu.VMEM((D, D), BF16),
                pltpu.VMEM((D + 16, F), BF16),
                pltpu.VMEM((D + 16, F), BF16),
                pltpu.VMEM((D + 16, F), BF16),
                pltpu.VMEM((D, 6 * D), BF16),
                pltpu.VMEM((6 * D, LANES), F32),
                pltpu.VMEM((D // 2 + KV, D), U32),
                pltpu.VMEM((D // 2, D), U32),
                pltpu.VMEM((NT, D + 16, LANES), F32),
                pltpu.VMEM((NT, LANES, LANES), F32),
                pltpu.VMEM((NT * NV, DH * 8, LANES), F32),
                pltpu.VMEM((KV, S), F32),
                pltpu.VMEM((NT + 1, D + 8, LANES), F32),
                pltpu.VMEM((NT + 1, H, LANES), F32),
                pltpu.VMEM((NMXU + 1, LANES, LANES), F32),
                pltpu.VMEM((POFF[-1], 64, LANES), U32),
                pltpu.VMEM((NU, POFF[-1], 64, 2 * LANES), U32),
                pltpu.VMEM((NU, 49, QD // 2, LANES), U32),
                *[pltpu.VMEM((253 * 16, LANES), F32)] * 3,
                pltpu.SMEM((1,), jnp.int32),
                pltpu.SemaphoreType.DMA((15,)),
            ],
            compiler_params=pltpu.CompilerParams(vmem_limit_bytes=120 * 2 ** 20),
            name="adaln_mqa_swiglu",
        )(c, A_wk.T, A_wv.T, A_x.reshape(S, D).T, A_wq, A_wo, B_w_gate, B_w_up, B_w_down.T, w_mod)
        return outT.T.reshape(1, S, D)

    return jax.jit(fn)


_kernel_fn = make()


@jax.jit
def pallas_adaLN_cond__grouped_kv_mqa__swiglu_ffn__prompt_kernel(
    A_x, A_wq, A_wk, A_wv, A_wo, B_x, B_w_gate, B_w_up, B_w_down, c, w_mod,
):
    return _kernel_fn(A_x, A_wq, A_wk, A_wv, A_wo, B_x, B_w_gate, B_w_up, B_w_down, c, w_mod)
```

```python
import functools
import math

import jax
import jax.numpy as jnp
from jax import lax
import jax.experimental.pallas as pl
import jax.experimental.pallas.tpu as pltpu

S, D, H, DH, F = 2048, 576, 32, 18, 4608
EPS = 1e-5
LANES = 128
NMXU = 4
NT = S // LANES
TB = 4 * LANES
NB = S // TB
HD, QD, QF = D // 2, D // 4, F // 4
NU = QF // LANES
KV = 24
SPARE = 16
BF16, F32, U32 = jnp.bfloat16, jnp.float32, jnp.uint32
NT_DIMS = (((1,), (1,)), ((), ()))
L_MIN, L_MAX, V_MAX = 2.0 ** -60, 2.0 ** 100, 2.0 ** 20

VPOS = ((0, 4, 10), (1, 6, 11), (2, 7, 13), (3, 9, 14))
NV = len(VPOS[0])
KEY_ORDER = [[g for g in range(16) if g not in v] + list(v) for v in VPOS]
NACC = 3


def _lhs7(a11, a12, a21, a22):
    return [a11 + a22, a21 + a22, a11, a22, a11 + a12, a21 - a11, a12 - a22]


def _rhs7(b11, b12, b21, b22, swap=False):
    if swap:
        b11, b12, b21, b22 = b12, b11, b22, b21
    return [b11 + b22, b11, b12 - b22, b21 - b11, b22, b11 + b12, b21 + b22]


def _out7(m, swap=False):
    c11, c12 = ((m[0] + m[3]) - m[4]) + m[6], m[2] + m[4]
    c21, c22 = m[1] + m[3], ((m[0] - m[1]) + m[2]) + m[5]
    return [c12, c11, c22, c21] if swap else [c11, c12, c21, c22]


SWAP = (False, False, True, False, True, True, True)
ORDER7 = (0, 3, 1, 2, 4, 5, 6)
ORDER49 = [7 * p + i for p in ORDER7 for i in ORDER7]


def _rhs49(b):
    outer = [_rhs7(*[b[2 * k1 + k2, 2 * j1 + j2] for k1 in range(2) for j1 in range(2)])
             for k2 in range(2) for j2 in range(2)]
    return [v for p in range(7) for v in _rhs7(*[x[p] for x in outer], swap=SWAP[p])]


def _out49(m):
    inner = [_out7([m[7 * p + i] for i in range(7)], swap=SWAP[p]) for p in range(7)]
    return {(n1 // 2 * 2 + n2 // 2, n1 % 2 * 2 + n2 % 2): v
            for n2 in range(4) for n1, v in enumerate(_out7([x[n2] for x in inner]))}


GU_CUTS = ((0, 192), (384, 64), (512, 64))
GU_STACK = (((0, 0),), ((1, 0),), ((0, 1), (1, 1)), ((0, 2), (1, 3)), ((0, 3), (1, 2)), ((0, 4), (1, 4)),
            ((0, 5), (2, 1)), ((0, 6), (2, 0)), ((1, 5), (2, 0)), ((1, 6), (2, 1)))
GU_DEPTH = [sum(GU_CUTS[part][1] for part, _ in stack) for stack in GU_STACK]
GU_INNER = [d > LANES for d in GU_DEPTH]
GU_PASS = [d // 2 if d > LANES else d for d in GU_DEPTH]
GU_OFF = [sum(7 if x else 2 for x in GU_INNER[:p]) for p in range(len(GU_STACK) + 1)]


def _gu_slab(p, r):
    first = GU_CUTS[GU_STACK[p][0][0]][1]
    return (*GU_STACK[p][r >= first], r - first * (r >= first))


def _gu_out(p):
    return [((p[0] + p[4]) - p[5]) + p[7], ((p[5] + p[3]) + p[1]) + p[9],
            ((p[4] + p[2]) + p[1]) + p[8], ((p[0] - p[2]) + p[3]) + p[6]]


def _same(*xs):
    return xs


def _dot(a, b):
    return jnp.dot(a, b, preferred_element_type=F32)


def _lead(ref, idx, rows):
    return pltpu.bitcast(ref.bitcast(U32)[(*idx, slice(0, rows // 2))], BF16)


class _Spread:
    def __init__(self, jobs, slots, zero_s):
        self.jobs, self.rate = list(jobs), sum(job[1] for job in jobs) / slots
        self.zero, self.credit = pl.multiple_of(zero_s[0], SPARE), 0.0

    def under(self, results):
        for m in range(0, results[0].shape[0], 8):
            self.credit += self.rate
            while self.jobs and self.credit > 0:
                src, cost, fn = self.jobs.pop(0)
                self.credit -= cost
                mark = pltpu.bitcast(results[len(self.jobs) % len(results)][m:m + 8], src.dtype)
                src[pl.ds(self.zero + src.shape[0] - SPARE, mark.shape[0]), 0:LANES] = mark
                fn()


def _kernel(c_hbm, wkT_hbm, wvT_hbm, xT_hbm, wq_hbm, wo_hbm, wg_hbm, wu_hbm, wdT_hbm, wmod_hbm,
            out_hbm,
            c_v, wkT_v, wvT_v, x_v, wq_v, wo_v, wg_v, wu_v, wdT_v, wmod_v,
            modc, wT, woT, q_s, k_s, kb_s, v_s, o_s, l_s, p_s, h2_s, wgu_s, wd_s, act_s,
            part0, part1, part2, zero_s, in_sems, out_sems):
    parts = (part0, part1, part2)
    cuts = (0, 5 * LANES, 2 * D, 14 * LANES, 6 * D)
    loads = [pltpu.make_async_copy(src, dst, in_sems.at[i]) for i, (src, dst) in enumerate(
        [(c_hbm, c_v), (wkT_hbm, wkT_v), (wvT_hbm, wvT_v), (wq_hbm, wq_v)]
        + [(wmod_hbm.at[:, lo:hi], wmod_v.at[:, lo:hi]) for lo, hi in zip(cuts, cuts[1:])]
        + [(wo_hbm, wo_v), (wg_hbm, wg_v.at[0:D]), (wu_hbm, wu_v.at[0:D]), (wdT_hbm, wdT_v.at[0:D])]
        + [(xT_hbm.at[:, pl.ds(b * TB, TB)], x_v.at[b]) for b in range(NB)])]
    cp_small, cp_wq, cp_mod, cp_late, cp_x = loads[0:3], loads[3], loads[4:6], loads[6:12], loads[12:]

    def out_copy(b, n):
        rows, col = pl.ds(n // 2 * HD, HD), n % 2 * (TB // 2)
        return pltpu.make_async_copy(
            x_v.at[b, rows, pl.ds(col, TB // 2)],
            out_hbm.at[rows, pl.ds(pl.multiple_of(b * TB + col, TB // 2), TB // 2)],
            out_sems.at[4 * b + n])

    for cp in cp_small + [cp_wq] + cp_mod + cp_x:
        cp.start()
    zero_s[0] = 0
    q_s[:, D:D + SPARE, :] = jnp.zeros((NT, SPARE, LANES), F32)
    p_s[...] = jnp.ones(p_s.shape, F32)
    for cp in cp_small:
        cp.wait()

    def mod_columns(part):
        scale, shift = (1.0, 1.0, 1.0, 0.5, 0.5, 2.0), (0.0, 1.0, 0.0, 0.0, 0.5, 0.0)
        lo, hi = cuts[part], cuts[part + 1]
        c = c_v[...].astype(F32)
        c = jnp.broadcast_to(c * jax.nn.sigmoid(c), (16, D)).astype(BF16)
        m = _dot(c, wmod_v[:, lo:hi])[0:1, :]
        col = lax.broadcasted_iota(jnp.int32, m.shape, 1) + lo
        for i in range(lo // D, -(-hi // D)):
            m = jnp.where((col >= i * D) & (col < (i + 1) * D), m * scale[i] + shift[i], m)
        modc[lo:hi, :] = jnp.broadcast_to(m, (LANES, hi - lo)).T

    pad = jnp.zeros((KV - DH, D), F32)
    wT[0:KV, :] = pltpu.bitcast(jnp.concatenate(
        [wkT_v[...].astype(F32), pad, wvT_v[...].astype(F32), pad], axis=0).astype(BF16), U32)
    cp_wq.wait()
    wT[KV:KV + D // 2, :] = pltpu.bitcast(wq_v[...].T, U32)
    for i, cp in enumerate(cp_mod):
        cp.wait()
        mod_columns(i)

    def qkv(b):
        hs = []
        for j in range(4):
            x = x_v[b, :, j * LANES:(j + 1) * LANES].astype(F32)
            x = x - jnp.sum(x, axis=0, keepdims=True) * (1.0 / D)
            var = jnp.sum(x * x, axis=0, keepdims=True) * (1.0 / D)
            hs.append(x * lax.rsqrt(var + EPS) * modc[D:2 * D, :] + modc[0:D, :])
        res = _dot(pltpu.bitcast(wT[...], BF16), jnp.concatenate(hs, axis=1).astype(BF16))
        for j in range(4):
            t = 4 * b + j
            blk = res[:, j * LANES:(j + 1) * LANES]
            q_s[t, 0:D, :] = blk[2 * KV:]
            k = blk[0:KV] * (DH ** -0.5 * math.log2(math.e))
            k = jnp.concatenate([k, jnp.zeros((LANES - KV, LANES), F32)], axis=0).T
            groups = [k[8 * (15 - g):8 * (16 - g)] for g in range(16)]
            k_s[t] = jnp.concatenate([groups[g] for g in KEY_ORDER[j]], axis=0)
            for r, g in enumerate(VPOS[j]):
                kb_s[t * NV + r] = jnp.concatenate(
                    [jnp.broadcast_to(groups[g][:, d:d + 1], (8, LANES)) for d in range(DH)], axis=0)
            row = lax.broadcasted_iota(jnp.int32, (KV, LANES), 0)
            v_s[:, t * LANES:(t + 1) * LANES] = jnp.where(row == DH, 1.0, blk[KV:2 * KV])

    cp_x[0].wait()
    qkv(0)
    for cp in cp_x[1:]:
        cp.wait()
    for b in range(1, NB):
        qkv(b)

    def weight_jobs(u):
        cols = [pl.ds(pl.multiple_of(j * QF + u * LANES, LANES), LANES) for j in range(4)]
        slots, jobs = {}, []

        def outer(w_v, where, combine, part_s, keys):
            new = combine(*[w_v[pl.ds(r, 16), cols[j]].astype(F32) for r, j in where])
            for key, v in zip(keys, new):
                part_s[pl.ds(16 * slots[key], 16), :] = v

        def inner(part_s, keys, combine, dst, index, r):
            for i, v in enumerate(combine(*[part_s[pl.ds(16 * slots[key], 16), :] for key in keys])):
                dst[(u, index[0] + i, *index[1:], pl.ds(r, 16))] = v.astype(BF16)

        for n, w_v in enumerate((wg_v, wu_v)):
            used = 0
            for part, (lo, size) in enumerate(GU_CUTS):
                combine = functools.partial(_rhs7, swap=part == 1) if part < 2 else _same
                for r in range(0, size, 16):
                    for j2 in range(2):
                        keys = [(n, part, i, r, j2) for i in range(7 if part < 2 else 2)]
                        slots.update((key, used + i) for i, key in enumerate(keys))
                        used += len(keys)
                        where = [(lo + k * size + r, 2 * j1 + j2)
                                 for k in range(2 if part < 2 else 1) for j1 in range(2)]
                        jobs.append((w_v, 32 if part < 2 else 8,
                                     functools.partial(outer, w_v, where, combine, parts[n], keys)))
            for p, depth in enumerate(GU_PASS):
                for r in range(0, depth, 16):
                    rows = (r, depth + r) if GU_INNER[p] else (r,)
                    keys = [(n, *_gu_slab(p, k), j2) for k in rows for j2 in range(2)]
                    jobs.append((parts[n], 17 if GU_INNER[p] else 6, functools.partial(
                        inner, parts[n], keys, _rhs7 if GU_INNER[p] else _same, wgu_s, (GU_OFF[p], n), r)))
        for r in range(0, QD, 16):
            for q in range(4):
                keys = [(2, p, r, q) for p in range(7)]
                slots.update((key, (r // 4 + q) * 7 + p) for p, key in enumerate(keys))
                where = [((2 * i1 + q // 2) * QD + r, 2 * j1 + q % 2) for i1 in range(2) for j1 in range(2)]
                jobs.append((wdT_v, 32, functools.partial(outer, wdT_v, where, _lhs7, parts[2], keys)))
        for r in range(0, QD, 16):
            for p in range(7):
                keys = [(2, p, r, q) for q in range(4)]
                jobs.append((parts[2], 17, functools.partial(inner, parts[2], keys, _lhs7, wd_s, (7 * p,), r)))
        return jobs

    NC = NT // NMXU

    def values(slot, h, c, ps, acc):
        o = [_dot(v_s[:, pl.ds((NMXU * c + j) * LANES, LANES)], p) for j, p in enumerate(ps)]
        o = (o[0] + o[1]) + (o[2] + o[3])
        acc = acc + o if c else o
        if c == NC - 1:
            l = acc[DH:DH + 1, :]
            l_s[slot, h:h + 1, :] = l
            r = pltpu.reciprocal(l, approx=True)
            o_s[slot, pl.ds(DH * h, KV), :] = acc * (r * (2.0 - l * r))
        return acc

    def carried(slot):
        return slot, H - 1, NC - 1, [p_s[j] for j in range(NMXU)], p_s[NMXU, 0:KV, :]

    def attention(t, jobs):
        side = _Spread(jobs, 50 * (16 - NV + 1), zero_s)

        def scores(q, q_rows, c):
            raw, ps = [], []
            for j in range(NMXU):
                kt, by_vpu = NMXU * c + j, list(range(NV))
                if side.jobs:
                    cut = 8 * (VPOS[j][by_vpu.pop(1)] - 1)
                    k = jnp.concatenate([k_s[kt, 0:cut, 0:32], k_s[kt, pl.ds(LANES - 8 * (NV - 1), 8), 0:32],
                                         k_s[kt, cut:LANES - 8 * NV, 0:32]], axis=0)
                else:
                    k = k_s[kt, 0:LANES - 8 * NV, 0:32]
                raw.append(_dot(k, q))
                p = jnp.exp2(raw[-1])
                blocks = [p[m:m + 8] for m in range(0, p.shape[0], 8)]
                for r in by_vpu:
                    s = None
                    for i, rows in enumerate(q_rows):
                        term = kb_s[kt * NV + r, pl.ds(i * NACC * 8, NACC * 8), :] * rows
                        s = s + term if i else term
                    blocks.insert(VPOS[j][r], jnp.exp2(jnp.sum(s.reshape(NACC, 8, LANES), axis=0)))
                ps.append(jnp.concatenate(blocks[::-1], axis=0))
            side.under(raw)
            return ps

        todo = carried(t)
        for h in range(H):
            q = q_s[t, pl.ds(DH * h, 32), :]
            q, rows = q.astype(BF16), [jnp.broadcast_to(q[d:d + 1], (8, LANES)) for d in range(DH)]
            rows = [jnp.concatenate(rows[d:d + NACC], axis=0) for d in range(0, DH, NACC)]
            for c in range(NC):
                ps = scores(q, rows, c)
                todo = (t + 1, h, c, ps, values(*todo))
        assert not side.jobs
        for j in range(NMXU):
            p_s[j] = todo[3][j]
        p_s[NMXU, 0:KV, :] = todo[4]

    @pl.loop(0, NT - NU)
    def _(t):
        @pl.when(t == 1)
        def _():
            for cp in cp_late:
                cp.start()

        attention(t, [])

    for cp in cp_late:
        cp.wait()

    @pl.loop(0, NU)
    def _(u):
        attention(NT - NU + u, weight_jobs(u))

    values(*carried(NT))

    for k2 in range(2):
        w = [wo_v[pl.ds((2 * k1 + k2) * LANES, LANES), :].T for k1 in range(2)]
        for r in range(0, HD, 16):
            blocks = [x[i * HD + r:i * HD + r + 16].astype(F32) for i in range(2) for x in w]
            for p, v in enumerate(_lhs7(*blocks)):
                woT[2 * p + k2, pl.ds(r, 16), :] = v.astype(BF16)
    w = wo_v[4 * LANES:D, :].T
    for i in range(2):
        woT[14 + i, :, 0:D - 4 * LANES] = w[i * HD:(i + 1) * HD]
    mod_columns(2)

    sums = l_s[1:NT + 1]
    unsafe = jnp.maximum(jnp.max(jnp.where((sums >= L_MIN) & (sums <= L_MAX), 0.0, 1.0)),
                         jnp.max(jnp.where(jnp.abs(v_s[...]) <= V_MAX, 0.0, 1.0)))

    @pl.when(unsafe > 0.0)
    def _():
        @pl.loop(0, NT * (H // 4))
        def _(n):
            t, base = n // (H // 4), pl.multiple_of(n % (H // 4) * (4 * DH), 8)
            q = q_s[t, pl.ds(base, 4 * DH + 16), :]
            q = jnp.concatenate([q[DH * i:DH * i + 32] for i in range(4)], axis=1).astype(BF16)
            k = jnp.concatenate([k_s[kt, pl.ds(8 * KEY_ORDER[kt % NMXU].index(g), 8), 0:32]
                                 for kt in range(NT) for g in range(15, -1, -1)], axis=0)
            s = _dot(k, q)
            o = _dot(v_s[...], jnp.exp2(s - jnp.max(s, axis=0, keepdims=True)).astype(BF16))
            o = o * (1.0 / o[DH:DH + 1, :])
            o_s[t + 1, pl.ds(base, 4 * DH), :] = jnp.concatenate(
                [o[0:DH, i * LANES:(i + 1) * LANES] for i in range(4)], axis=0)

    def norm_jobs(b):
        stats, jobs, hT = {}, [], parts[0]

        def total(j, r):
            part = jnp.sum(q_s[4 * b + j, pl.ds(r, 96), :].reshape(12, 8, LANES), axis=0)
            stats["s", j] = stats["s", j] + part if r else part

        def variance(j, r):
            if r == 0:
                stats["m", j] = jnp.sum(stats["s", j], axis=0, keepdims=True) * (1.0 / D)
            d = q_s[4 * b + j, pl.ds(r, 48), :] - stats["m", j]
            part = jnp.sum((d * d).reshape(6, 8, LANES), axis=0)
            stats["v", j] = stats["v", j] + part if r else part

        def normalise(j, r):
            if r == 0:
                stats["r", j] = lax.rsqrt(jnp.sum(stats["v", j], axis=0, keepdims=True) * (1.0 / D) + EPS)
            d = q_s[4 * b + j, pl.ds(r, 48), :] - stats["m", j]
            hT[pl.ds(j * D + r, 48), :] = (
                d * stats["r", j] * modc[pl.ds(4 * D + r, 48), :] + modc[pl.ds(3 * D + r, 48), :])

        def slab(p, r, i2):
            part, i, r = _gu_slab(p, r)
            lo, size = GU_CUTS[part]
            h = [hT[pl.ds((2 * i1 + i2) * D + lo + k * size + r, 16), :]
                 for i1 in range(2) for k in range(2 if part < 2 else 1)]
            v = _lhs7(*h)[i] if part < 2 else h[p in (6, 8)]
            return -v if part == 1 and p in (2, 5) else v

        def factor(p, i):
            depth = GU_PASS[p]
            rows = [_lhs7(*[slab(p, k * depth + r, i2) for i2 in range(2) for k in range(2)])[i]
                    if GU_INNER[p] else slab(p, r, i) for r in range(0, depth, 16)]
            h2_s[GU_OFF[p] + i, :, 0:depth] = pltpu.bitcast(jnp.concatenate(rows, axis=0).astype(BF16).T, U32)

        for j in range(4):
            for fn, step in ((total, 96), (variance, 48), (normalise, 48)):
                jobs += [(q_s.at[4 * b + j], 20, functools.partial(fn, j, r)) for r in range(0, D, step)]
        for p in range(len(GU_STACK)):
            jobs += [(hT, 60, functools.partial(factor, p, i)) for i in range(GU_OFF[p + 1] - GU_OFF[p])]
        return jobs

    for b in range(NB):
        def heads(k, j):
            return o_s[4 * b + j + 1, k * LANES:min(D, (k + 1) * LANES), :]

        m = [{}, {}]
        for p in ORDER7:
            for j2 in range(2):
                v = [_rhs7(*[heads(2 * k1 + k2, 2 * j1 + j2) for k1 in range(2) for j1 in range(2)])[p]
                     for k2 in range(2)]
                m[j2][p] = _dot(woT[2 * p], v[0].astype(BF16)) + _dot(woT[2 * p + 1], v[1].astype(BF16))
            if b:
                side.under([m[0][p], m[1][p]])
        for j2 in range(2):
            for n, v in enumerate(_out7(m[j2])):
                rows, j = pl.ds(n // 2 * HD, HD), n % 2 * 2 + j2
                v = v + _dot(woT[14 + n // 2, :, 0:D - 4 * LANES], heads(4, j).astype(BF16))
                x = x_v[b, rows, j * LANES:(j + 1) * LANES].astype(F32)
                q_s[4 * b + j, rows, :] = x + modc[pl.ds(2 * D + rows.start, HD), :] * v
        if b == 0:
            mod_columns(3)
            side = _Spread(norm_jobs(0), 19 * HD // 8, zero_s)
    assert not side.jobs

    def gate_up(u):
        def mm(p, il, ir):
            w = [_lead(wgu_s, (u, GU_OFF[p] + ir, n), GU_PASS[p]) for n in range(2)]
            return _dot(pltpu.bitcast(h2_s[GU_OFF[p] + il, :, 0:GU_PASS[p]], BF16), jnp.concatenate(w, axis=1))

        prod = {p: _out7({i: mm(p, i, i) for i in ORDER7}) for p in (0, 4, 5, 7, 2, 3, 6)}
        prod[1], prod[8], prod[9] = zip(*[[mm(p, n // 2, n % 2) for p in (1, 8, 9)] for n in range(4)])
        act = {}
        for n2 in range(4):
            for n1, v in enumerate(_gu_out([prod[p][n2] for p in range(len(GU_STACK))])):
                g, up = v[:, :LANES], v[:, LANES:]
                act[n1 % 2 * 2 + n2 % 2, n1 // 2 * 2 + n2 // 2] = (g * jnp.tanh(g) + g) * up
        for p, v in enumerate(_rhs49(act)):
            act_s[u, p] = v.astype(BF16)

    def down(u, p):
        return lax.dot_general(_lead(wd_s, (u, p), QD), _lead(act_s, (u, p), LANES), NT_DIMS,
                               preferred_element_type=F32)

    @pl.loop(0, NB)
    def _(b):
        @pl.loop(0, NU // 3)
        def _(i):
            for n in range(3):
                gate_up(3 * i + n)

        side = _Spread(norm_jobs(jnp.minimum(b + 1, NB - 1)), 80 * QD // 8, zero_s)
        m = {}
        for n in range(0, len(ORDER49), NMXU):
            m.update((p, down(NU - 1, p)) for p in ORDER49[n:n + NMXU])
            for p in ORDER49[n:n + NMXU]:
                for u in range(0, NU - 1, NMXU):
                    v = [down(u + j, p) for j in range(NMXU)]
                    v = [v[0] + v[1], v[2] + v[3]]
                    side.under(v)
                    m[p] = m[p] + (v[0] + v[1])
        assert not side.jobs
        y = _out49(m)
        for n in (2, 1, 3, 0):
            for i in range(n // 2 * 2, n // 2 * 2 + 2):
                rows = pl.ds(i * QD, QD)
                for j in range(n % 2 * 2, n % 2 * 2 + 2):
                    x_v[b, rows, j * LANES:(j + 1) * LANES] = (
                        q_s[4 * b + j, rows, :] + modc[pl.ds(5 * D + i * QD, QD), :] * y[i, j]).astype(BF16)
            out_copy(b, n).start()

    for b in range(NB):
        for n in (2, 1, 3, 0):
            out_copy(b, n).wait()


@jax.jit
def pallas_adaLN_cond__grouped_kv_mqa__swiglu_ffn__prompt_kernel(
    A_x: jax.Array,
    A_wq: jax.Array,
    A_wk: jax.Array,
    A_wv: jax.Array,
    A_wo: jax.Array,
    B_x: jax.Array,
    B_w_gate: jax.Array,
    B_w_up: jax.Array,
    B_w_down: jax.Array,
    c: jax.Array,
    w_mod: jax.Array,
):
    del B_x
    hbm = pl.BlockSpec(memory_space=pl.ANY)
    outT = pl.pallas_call(
        _kernel,
        out_shape=jax.ShapeDtypeStruct((D, S), BF16),
        in_specs=[hbm] * 10,
        out_specs=hbm,
        scratch_shapes=[
            pltpu.VMEM((1, D), BF16),
            pltpu.VMEM((DH, D), BF16),
            pltpu.VMEM((DH, D), BF16),
            pltpu.VMEM((NB, D, TB), BF16),
            pltpu.VMEM((D, D), BF16),
            pltpu.VMEM((D, D), BF16),
            pltpu.VMEM((D + SPARE, F), BF16),
            pltpu.VMEM((D + SPARE, F), BF16),
            pltpu.VMEM((D + SPARE, F), BF16),
            pltpu.VMEM((D, 6 * D), BF16),
            pltpu.VMEM((6 * D, LANES), F32),
            pltpu.VMEM((KV + D // 2, D), U32),
            pltpu.VMEM((16, HD, LANES), BF16),
            pltpu.VMEM((NT, D + SPARE, LANES), F32),
            pltpu.VMEM((NT, LANES, LANES), F32),
            pltpu.VMEM((NT * NV, DH * 8, LANES), F32),
            pltpu.VMEM((KV, S), F32),
            pltpu.VMEM((NT + 1, D + 8, LANES), F32),
            pltpu.VMEM((NT + 1, H, LANES), F32),
            pltpu.VMEM((NMXU + 1, LANES, LANES), F32),
            pltpu.VMEM((GU_OFF[-1], LANES // 2, LANES), U32),
            pltpu.VMEM((NU, GU_OFF[-1], 2, LANES, LANES), BF16),
            pltpu.VMEM((NU, 49, QD, LANES), BF16),
            pltpu.VMEM((NU, 49, LANES, LANES), BF16),
            *[pltpu.VMEM((252 * 16 + SPARE, LANES), F32)] * 3,
            pltpu.SMEM((1,), jnp.int32),
            pltpu.SemaphoreType.DMA((12 + NB,)),
            pltpu.SemaphoreType.DMA((4 * NB,)),
        ],
        compiler_params=pltpu.CompilerParams(vmem_limit_bytes=120 * 2 ** 20),
        name="adaln_mqa_swiglu",
    )(c, A_wk.T, A_wv.T, A_x.reshape(S, D).T, A_wq, A_wo, B_w_gate, B_w_up, B_w_down.T, w_mod)
    return outT.T.reshape(1, S, D)
```

```python
import functools
import math

import jax
import jax.numpy as jnp
from jax import lax
import jax.experimental.pallas as pl
import jax.experimental.pallas.tpu as pltpu

S, D, H, DH, F = 2048, 576, 32, 18, 4608
EPS = 1e-5
LANES = 128
NMXU = 4
NT = S // LANES
TB = 4 * LANES
NB = S // TB
HD, QD, QF = D // 2, D // 4, F // 4
NU = QF // LANES
KV = 24
SPARE = 16
BF16, F32, U32 = jnp.bfloat16, jnp.float32, jnp.uint32
NT_DIMS = (((1,), (1,)), ((), ()))
L_MIN, L_MAX, V_MAX = 2.0 ** -60, 2.0 ** 100, 2.0 ** 20

VPOS = ((0, 4, 10), (1, 6, 11), (2, 7, 13), (3, 9, 14))
NV = len(VPOS[0])
KEY_ORDER = [[g for g in range(16) if g not in v] + list(v) for v in VPOS]
NACC = 3


def _lhs7(a11, a12, a21, a22):
    return [a11 + a22, a21 + a22, a11, a22, a11 + a12, a21 - a11, a12 - a22]


def _rhs7(b11, b12, b21, b22, swap=False):
    if swap:
        b11, b12, b21, b22 = b12, b11, b22, b21
    return [b11 + b22, b11, b12 - b22, b21 - b11, b22, b11 + b12, b21 + b22]


def _out7(m, swap=False):
    c11, c12 = ((m[0] + m[3]) - m[4]) + m[6], m[2] + m[4]
    c21, c22 = m[1] + m[3], ((m[0] - m[1]) + m[2]) + m[5]
    return [c12, c11, c22, c21] if swap else [c11, c12, c21, c22]


SWAP = (False, False, True, False, True, True, True)
ORDER7 = (0, 3, 1, 2, 4, 5, 6)
ORDER49 = [7 * p + i for p in ORDER7 for i in ORDER7]


def _rhs49(b):
    outer = [_rhs7(*[b[2 * k1 + k2, 2 * j1 + j2] for k1 in range(2) for j1 in range(2)])
             for k2 in range(2) for j2 in range(2)]
    return [v for p in range(7) for v in _rhs7(*[x[p] for x in outer], swap=SWAP[p])]


def _out49(m):
    inner = [_out7([m[7 * p + i] for i in range(7)], swap=SWAP[p]) for p in range(7)]
    return {(n1 // 2 * 2 + n2 // 2, n1 % 2 * 2 + n2 % 2): v
            for n2 in range(4) for n1, v in enumerate(_out7([x[n2] for x in inner]))}


GU_CUTS = ((0, 192), (384, 64), (512, 64))
GU_STACK = (((0, 0),), ((1, 0),), ((0, 1), (1, 1)), ((0, 2), (1, 3)), ((0, 3), (1, 2)), ((0, 4), (1, 4)),
            ((0, 5), (2, 1)), ((0, 6), (2, 0)), ((1, 5), (2, 0)), ((1, 6), (2, 1)))
GU_DEPTH = [sum(GU_CUTS[part][1] for part, _ in stack) for stack in GU_STACK]
GU_INNER = [d > LANES for d in GU_DEPTH]
GU_PASS = [d // 2 if d > LANES else d for d in GU_DEPTH]
GU_OFF = [sum(7 if x else 2 for x in GU_INNER[:p]) for p in range(len(GU_STACK) + 1)]


def _gu_slab(p, r):
    first = GU_CUTS[GU_STACK[p][0][0]][1]
    return (*GU_STACK[p][r >= first], r - first * (r >= first))


def _gu_out(p):
    return [((p[0] + p[4]) - p[5]) + p[7], ((p[5] + p[3]) + p[1]) + p[9],
            ((p[4] + p[2]) + p[1]) + p[8], ((p[0] - p[2]) + p[3]) + p[6]]


def _same(*xs):
    return xs


def _dot(a, b):
    return jnp.dot(a, b, preferred_element_type=F32)


class _Spread:
    def __init__(self, jobs, slots, zero_s):
        self.jobs, self.rate = list(jobs), sum(job[1] for job in jobs) / slots
        self.zero, self.credit = pl.multiple_of(zero_s[0], SPARE), 0.0

    def under(self, results):
        for m in range(0, results[0].shape[0], 8):
            self.credit += self.rate
            while self.jobs and self.credit > 0:
                src, cost, fn = self.jobs.pop(0)
                self.credit -= cost
                mark = pltpu.bitcast(results[len(self.jobs) % len(results)][m:m + 8], src.dtype)
                src[pl.ds(self.zero + src.shape[0] - SPARE, mark.shape[0]), 0:LANES] = mark
                fn()


def _kernel(c_hbm, wkT_hbm, wvT_hbm, xT_hbm, wq_hbm, wo_hbm, wg_hbm, wu_hbm, wdT_hbm, wmod_hbm,
            out_hbm,
            c_v, wkT_v, wvT_v, x_v, wq_v, wo_v, wg_v, wu_v, wdT_v, wmod_v,
            modc, wT, woT, q_s, k_s, kb_s, v_s, o_s, l_s, p_s, h2_s, wgu_s, wd_s, act_s,
            part0, part1, part2, zero_s, in_sems, out_sems):
    parts = (part0, part1, part2)
    cuts = (0, 5 * LANES, 2 * D, 14 * LANES, 6 * D)
    loads = [pltpu.make_async_copy(src, dst, in_sems.at[i]) for i, (src, dst) in enumerate(
        [(c_hbm, c_v), (wkT_hbm, wkT_v), (wvT_hbm, wvT_v), (wq_hbm, wq_v)]
        + [(wmod_hbm.at[:, lo:hi], wmod_v.at[:, lo:hi]) for lo, hi in zip(cuts, cuts[1:])]
        + [(wo_hbm, wo_v), (wg_hbm, wg_v.at[0:D]), (wu_hbm, wu_v.at[0:D]), (wdT_hbm, wdT_v.at[0:D])]
        + [(xT_hbm.at[:, pl.ds(b * TB, TB)], x_v.at[b]) for b in range(NB)])]
    cp_small, cp_wq, cp_mod, cp_late, cp_x = loads[0:3], loads[3], loads[4:6], loads[6:12], loads[12:]

    def out_copy(b, n):
        rows, col = pl.ds(n // 2 * HD, HD), n % 2 * (TB // 2)
        return pltpu.make_async_copy(
            x_v.at[b, rows, pl.ds(col, TB // 2)],
            out_hbm.at[rows, pl.ds(pl.multiple_of(b * TB + col, TB // 2), TB // 2)],
            out_sems.at[4 * b + n])

    for cp in cp_small + [cp_wq] + cp_mod + cp_x:
        cp.start()
    zero_s[0] = 0
    q_s[:, D:D + SPARE, :] = jnp.zeros((NT, SPARE, LANES), F32)
    p_s[...] = jnp.ones(p_s.shape, F32)
    for cp in cp_small:
        cp.wait()

    def mod_columns(part):
        scale, shift = (1.0, 1.0, 1.0, 0.5, 0.5, 2.0), (0.0, 1.0, 0.0, 0.0, 0.5, 0.0)
        lo, hi = cuts[part], cuts[part + 1]
        c = c_v[...].astype(F32)
        c = jnp.broadcast_to(c * jax.nn.sigmoid(c), (16, D)).astype(BF16)
        m = _dot(c, wmod_v[:, lo:hi])[0:1, :]
        col = lax.broadcasted_iota(jnp.int32, m.shape, 1) + lo
        for i in range(lo // D, -(-hi // D)):
            m = jnp.where((col >= i * D) & (col < (i + 1) * D), m * scale[i] + shift[i], m)
        modc[lo:hi, :] = jnp.broadcast_to(m, (LANES, hi - lo)).T

    pad = jnp.zeros((KV - DH, D), F32)
    wT[0:KV, :] = pltpu.bitcast(jnp.concatenate(
        [wkT_v[...].astype(F32), pad, wvT_v[...].astype(F32), pad], axis=0).astype(BF16), U32)
    cp_wq.wait()
    wT[KV:KV + D // 2, :] = pltpu.bitcast(wq_v[...].T, U32)
    for i, cp in enumerate(cp_mod):
        cp.wait()
        mod_columns(i)

    def qkv(b):
        hs = []
        for j in range(4):
            x = x_v[b, :, j * LANES:(j + 1) * LANES].astype(F32)
            x = x - jnp.sum(x, axis=0, keepdims=True) * (1.0 / D)
            var = jnp.sum(x * x, axis=0, keepdims=True) * (1.0 / D)
            hs.append(x * lax.rsqrt(var + EPS) * modc[D:2 * D, :] + modc[0:D, :])
        res = _dot(pltpu.bitcast(wT[...], BF16), jnp.concatenate(hs, axis=1).astype(BF16))
        for j in range(4):
            t = 4 * b + j
            blk = res[:, j * LANES:(j + 1) * LANES]
            q_s[t, 0:D, :] = blk[2 * KV:]
            k = blk[0:KV] * (DH ** -0.5 * math.log2(math.e))
            k = jnp.concatenate([k, jnp.zeros((LANES - KV, LANES), F32)], axis=0).T
            groups = [k[8 * (15 - g):8 * (16 - g)] for g in range(16)]
            k_s[t] = jnp.concatenate([groups[g] for g in KEY_ORDER[j]], axis=0)
            for r, g in enumerate(VPOS[j]):
                kb_s[t * NV + r] = jnp.concatenate(
                    [jnp.broadcast_to(groups[g][:, d:d + 1], (8, LANES)) for d in range(DH)], axis=0)
            row = lax.broadcasted_iota(jnp.int32, (KV, LANES), 0)
            v_s[:, t * LANES:(t + 1) * LANES] = jnp.where(row == DH, 1.0, blk[KV:2 * KV])

    cp_x[0].wait()
    qkv(0)
    for cp in cp_x[1:]:
        cp.wait()
    for b in range(1, NB):
        qkv(b)

    def weight_jobs(u):
        cols = [pl.ds(pl.multiple_of(j * QF + u * LANES, LANES), LANES) for j in range(4)]
        slots, jobs = {}, []

        def outer(w_v, where, combine, part_s, keys):
            new = combine(*[w_v[pl.ds(r, 16), cols[j]].astype(F32) for r, j in where])
            for key, v in zip(keys, new):
                part_s[pl.ds(16 * slots[key], 16), :] = v

        def inner(part_s, keys, combine, dst, index, r):
            for i, v in enumerate(combine(*[part_s[pl.ds(16 * slots[key], 16), :] for key in keys])):
                dst[(u, index[0] + i, *index[1:], pl.ds(r, 16))] = v.astype(BF16)

        for n, w_v in enumerate((wg_v, wu_v)):
            used = 0
            for part, (lo, size) in enumerate(GU_CUTS):
                combine = functools.partial(_rhs7, swap=part == 1) if part < 2 else _same
                for r in range(0, size, 16):
                    for j2 in range(2):
                        keys = [(n, part, i, r, j2) for i in range(7 if part < 2 else 2)]
                        slots.update((key, used + i) for i, key in enumerate(keys))
                        used += len(keys)
                        where = [(lo + k * size + r, 2 * j1 + j2)
                                 for k in range(2 if part < 2 else 1) for j1 in range(2)]
                        jobs.append((w_v, 32 if part < 2 else 8,
                                     functools.partial(outer, w_v, where, combine, parts[n], keys)))
            for p, depth in enumerate(GU_PASS):
                for r in range(0, depth, 16):
                    rows = (r, depth + r) if GU_INNER[p] else (r,)
                    keys = [(n, *_gu_slab(p, k), j2) for k in rows for j2 in range(2)]
                    jobs.append((parts[n], 17 if GU_INNER[p] else 6, functools.partial(
                        inner, parts[n], keys, _rhs7 if GU_INNER[p] else _same, wgu_s, (GU_OFF[p], n), r)))
        for r in range(0, QD, 16):
            for q in range(4):
                keys = [(2, p, r, q) for p in range(7)]
                slots.update((key, (r // 4 + q) * 7 + p) for p, key in enumerate(keys))
                where = [((2 * i1 + q // 2) * QD + r, 2 * j1 + q % 2) for i1 in range(2) for j1 in range(2)]
                jobs.append((wdT_v, 32, functools.partial(outer, wdT_v, where, _lhs7, parts[2], keys)))
        for r in range(0, QD, 16):
            for p in range(7):
                keys = [(2, p, r, q) for q in range(4)]
                jobs.append((parts[2], 17, functools.partial(inner, parts[2], keys, _lhs7, wd_s, (7 * p,), r)))
        return jobs

    NC = NT // NMXU

    def values(slot, h, c, ps, acc):
        o = [_dot(v_s[:, pl.ds((NMXU * c + j) * LANES, LANES)], p) for j, p in enumerate(ps)]
        o = (o[0] + o[1]) + (o[2] + o[3])
        acc = acc + o if c else o
        if c == NC - 1:
            l = acc[DH:DH + 1, :]
            l_s[slot, h:h + 1, :] = l
            r = pltpu.reciprocal(l, approx=True)
            o_s[slot, pl.ds(DH * h, KV), :] = acc * (r * (2.0 - l * r))
        return acc

    def carried(slot):
        return slot, H - 1, NC - 1, [p_s[j] for j in range(NMXU)], p_s[NMXU, 0:KV, :]

    def attention(t, jobs):
        side = _Spread(jobs, 50 * (16 - NV + 1), zero_s)

        def scores(q, q_rows, c):
            raw, ps = [], []
            for j in range(NMXU):
                kt, by_vpu = NMXU * c + j, list(range(NV))
                if side.jobs:
                    cut = 8 * (VPOS[j][by_vpu.pop(1)] - 1)
                    k = jnp.concatenate([k_s[kt, 0:cut, 0:32], k_s[kt, pl.ds(LANES - 8 * (NV - 1), 8), 0:32],
                                         k_s[kt, cut:LANES - 8 * NV, 0:32]], axis=0)
                else:
                    k = k_s[kt, 0:LANES - 8 * NV, 0:32]
                raw.append(_dot(k, q))
                p = jnp.exp2(raw[-1])
                blocks = [p[m:m + 8] for m in range(0, p.shape[0], 8)]
                for r in by_vpu:
                    s = None
                    for i, rows in enumerate(q_rows):
                        term = kb_s[kt * NV + r, pl.ds(i * NACC * 8, NACC * 8), :] * rows
                        s = s + term if i else term
                    blocks.insert(VPOS[j][r], jnp.exp2(jnp.sum(s.reshape(NACC, 8, LANES), axis=0)))
                ps.append(jnp.concatenate(blocks[::-1], axis=0))
            side.under(raw)
            return ps

        todo = carried(t)
        for h in range(H):
            q = q_s[t, pl.ds(DH * h, 32), :]
            q, rows = q.astype(BF16), [jnp.broadcast_to(q[d:d + 1], (8, LANES)) for d in range(DH)]
            rows = [jnp.concatenate(rows[d:d + NACC], axis=0) for d in range(0, DH, NACC)]
            for c in range(NC):
                ps = scores(q, rows, c)
                todo = (t + 1, h, c, ps, values(*todo))
        assert not side.jobs
        for j in range(NMXU):
            p_s[j] = todo[3][j]
        p_s[NMXU, 0:KV, :] = todo[4]

    @pl.loop(0, NT - NU)
    def _(t):
        @pl.when(t == 1)
        def _():
            for cp in cp_late:
                cp.start()

        attention(t, [])

    for cp in cp_late:
        cp.wait()

    @pl.loop(0, NU)
    def _(u):
        attention(NT - NU + u, weight_jobs(u))

    values(*carried(NT))

    for k2 in range(2):
        w = [wo_v[pl.ds((2 * k1 + k2) * LANES, LANES), :].T for k1 in range(2)]
        for r in range(0, HD, 16):
            blocks = [x[i * HD + r:i * HD + r + 16].astype(F32) for i in range(2) for x in w]
            for p, v in enumerate(_lhs7(*blocks)):
                woT[2 * p + k2, pl.ds(r, 16), :] = v.astype(BF16)
    w = wo_v[4 * LANES:D, :].T
    for i in range(2):
        woT[14 + i, :, 0:D - 4 * LANES] = w[i * HD:(i + 1) * HD]
    mod_columns(2)

    sums = l_s[1:NT + 1]
    unsafe = jnp.maximum(jnp.max(jnp.where((sums >= L_MIN) & (sums <= L_MAX), 0.0, 1.0)),
                         jnp.max(jnp.where(jnp.abs(v_s[...]) <= V_MAX, 0.0, 1.0)))

    @pl.when(unsafe > 0.0)
    def _():
        @pl.loop(0, NT * (H // 4))
        def _(n):
            t, base = n // (H // 4), pl.multiple_of(n % (H // 4) * (4 * DH), 8)
            q = q_s[t, pl.ds(base, 4 * DH + 16), :]
            q = jnp.concatenate([q[DH * i:DH * i + 32] for i in range(4)], axis=1).astype(BF16)
            k = jnp.concatenate([k_s[kt, pl.ds(8 * KEY_ORDER[kt % NMXU].index(g), 8), 0:32]
                                 for kt in range(NT) for g in range(15, -1, -1)], axis=0)
            s = _dot(k, q)
            o = _dot(v_s[...], jnp.exp2(s - jnp.max(s, axis=0, keepdims=True)).astype(BF16))
            o = o * (1.0 / o[DH:DH + 1, :])
            o_s[t + 1, pl.ds(base, 4 * DH), :] = jnp.concatenate(
                [o[0:DH, i * LANES:(i + 1) * LANES] for i in range(4)], axis=0)

    def norm_jobs(b):
        stats, jobs, hT = {}, [], parts[0]

        def total(j, r):
            part = jnp.sum(q_s[4 * b + j, pl.ds(r, 96), :].reshape(12, 8, LANES), axis=0)
            stats["s", j] = stats["s", j] + part if r else part

        def variance(j, r):
            if r == 0:
                stats["m", j] = jnp.sum(stats["s", j], axis=0, keepdims=True) * (1.0 / D)
            d = q_s[4 * b + j, pl.ds(r, 48), :] - stats["m", j]
            part = jnp.sum((d * d).reshape(6, 8, LANES), axis=0)
            stats["v", j] = stats["v", j] + part if r else part

        def normalise(j, r):
            if r == 0:
                stats["r", j] = lax.rsqrt(jnp.sum(stats["v", j], axis=0, keepdims=True) * (1.0 / D) + EPS)
            d = q_s[4 * b + j, pl.ds(r, 48), :] - stats["m", j]
            hT[pl.ds(j * D + r, 48), :] = (
                d * stats["r", j] * modc[pl.ds(4 * D + r, 48), :] + modc[pl.ds(3 * D + r, 48), :])

        def slab(p, r, i2):
            part, i, r = _gu_slab(p, r)
            lo, size = GU_CUTS[part]
            h = [hT[pl.ds((2 * i1 + i2) * D + lo + k * size + r, 16), :]
                 for i1 in range(2) for k in range(2 if part < 2 else 1)]
            v = _lhs7(*h)[i] if part < 2 else h[p in (6, 8)]
            return -v if part == 1 and p in (2, 5) else v

        def factor(p, i):
            depth = GU_PASS[p]
            rows = [_lhs7(*[slab(p, k * depth + r, i2) for i2 in range(2) for k in range(2)])[i]
                    if GU_INNER[p] else slab(p, r, i) for r in range(0, depth, 16)]
            h2_s[GU_OFF[p] + i, :, 0:depth] = pltpu.bitcast(jnp.concatenate(rows, axis=0).astype(BF16).T, U32)

        for j in range(4):
            for fn, step in ((total, 96), (variance, 48), (normalise, 48)):
                jobs += [(q_s.at[4 * b + j], 20, functools.partial(fn, j, r)) for r in range(0, D, step)]
        for p in range(len(GU_STACK)):
            jobs += [(hT, 60, functools.partial(factor, p, i)) for i in range(GU_OFF[p + 1] - GU_OFF[p])]
        return jobs

    for b in range(NB):
        def heads(k, j):
            return o_s[4 * b + j + 1, k * LANES:min(D, (k + 1) * LANES), :]

        m = [{}, {}]
        for p in ORDER7:
            for j2 in range(2):
                v = [_rhs7(*[heads(2 * k1 + k2, 2 * j1 + j2) for k1 in range(2) for j1 in range(2)])[p]
                     for k2 in range(2)]
                m[j2][p] = _dot(woT[2 * p], v[0].astype(BF16)) + _dot(woT[2 * p + 1], v[1].astype(BF16))
            if b:
                side.under([m[0][p], m[1][p]])
        for j2 in range(2):
            for n, v in enumerate(_out7(m[j2])):
                rows, j = pl.ds(n // 2 * HD, HD), n % 2 * 2 + j2
                v = v + _dot(woT[14 + n // 2, :, 0:D - 4 * LANES], heads(4, j).astype(BF16))
                x = x_v[b, rows, j * LANES:(j + 1) * LANES].astype(F32)
                q_s[4 * b + j, rows, :] = x + modc[pl.ds(2 * D + rows.start, HD), :] * v
        if b == 0:
            mod_columns(3)
            side = _Spread(norm_jobs(0), 19 * HD // 8, zero_s)
    assert not side.jobs

    def gate_up(u):
        def mm(p, il, ir):
            w = [wgu_s[u, GU_OFF[p] + ir, n, 0:GU_PASS[p], :] for n in range(2)]
            return _dot(pltpu.bitcast(h2_s[GU_OFF[p] + il, :, 0:GU_PASS[p]], BF16), jnp.concatenate(w, axis=1))

        deep = (0, 4, 5, 7, 2, 3, 6)
        plain = [[(p, n) for p in (1, 8, 9)] for n in range(4)]
        order = ([(p, i) for p in deep for i in ORDER7[:5]] + plain[1] + [(p, 6) for p in deep] + plain[0]
                 + plain[2] + [(p, 5) for p in deep] + plain[3])
        m = {(p, i): mm(p, i, i) if GU_INNER[p] else mm(p, i // 2, i % 2) for p, i in order}
        prod = [_out7([m[p, i] for i in range(7)]) if GU_INNER[p] else [m[p, n] for n in range(4)]
                for p in range(len(GU_STACK))]
        act = {}
        for n2 in range(4):
            for n1, v in enumerate(_gu_out([x[n2] for x in prod])):
                g, up = v[:, :LANES], v[:, LANES:]
                act[n1 % 2 * 2 + n2 % 2, n1 // 2 * 2 + n2 // 2] = (g * jnp.tanh(g) + g) * up
        for p, v in enumerate(_rhs49(act)):
            act_s[u, p] = v.astype(BF16)

    def down(u, p):
        return lax.dot_general(wd_s[u, p], act_s[u, p], NT_DIMS, preferred_element_type=F32)

    @pl.loop(0, NB)
    def _(b):
        @pl.loop(0, NU // 3)
        def _(i):
            for n in range(3):
                gate_up(3 * i + n)

        side = _Spread(norm_jobs(jnp.minimum(b + 1, NB - 1)), 80 * QD // 8, zero_s)
        m = {}
        for n in range(0, len(ORDER49), NMXU):
            m.update((p, down(NU - 1, p)) for p in ORDER49[n:n + NMXU])
            for p in ORDER49[n:n + NMXU]:
                for u in range(0, NU - 1, NMXU):
                    v = [down(u + j, p) for j in range(NMXU)]
                    v = [v[0] + v[1], v[2] + v[3]]
                    side.under(v)
                    m[p] = m[p] + (v[0] + v[1])
        assert not side.jobs
        y = _out49(m)
        for n in (2, 1, 3, 0):
            for i in range(n // 2 * 2, n // 2 * 2 + 2):
                rows = pl.ds(i * QD, QD)
                for j in range(n % 2 * 2, n % 2 * 2 + 2):
                    x_v[b, rows, j * LANES:(j + 1) * LANES] = (
                        q_s[4 * b + j, rows, :] + modc[pl.ds(5 * D + i * QD, QD), :] * y[i, j]).astype(BF16)
            out_copy(b, n).start()

    for b in range(NB):
        for n in (2, 1, 3, 0):
            out_copy(b, n).wait()


@jax.jit
def pallas_adaLN_cond__grouped_kv_mqa__swiglu_ffn__prompt_kernel(
    A_x: jax.Array,
    A_wq: jax.Array,
    A_wk: jax.Array,
    A_wv: jax.Array,
    A_wo: jax.Array,
    B_x: jax.Array,
    B_w_gate: jax.Array,
    B_w_up: jax.Array,
    B_w_down: jax.Array,
    c: jax.Array,
    w_mod: jax.Array,
):
    del B_x
    hbm = pl.BlockSpec(memory_space=pl.ANY)
    outT = pl.pallas_call(
        _kernel,
        out_shape=jax.ShapeDtypeStruct((D, S), BF16),
        in_specs=[hbm] * 10,
        out_specs=hbm,
        scratch_shapes=[
            pltpu.VMEM((1, D), BF16),
            pltpu.VMEM((DH, D), BF16),
            pltpu.VMEM((DH, D), BF16),
            pltpu.VMEM((NB, D, TB), BF16),
            pltpu.VMEM((D, D), BF16),
            pltpu.VMEM((D, D), BF16),
            pltpu.VMEM((D + SPARE, F), BF16),
            pltpu.VMEM((D + SPARE, F), BF16),
            pltpu.VMEM((D + SPARE, F), BF16),
            pltpu.VMEM((D, 6 * D), BF16),
            pltpu.VMEM((6 * D, LANES), F32),
            pltpu.VMEM((KV + D // 2, D), U32),
            pltpu.VMEM((16, HD, LANES), BF16),
            pltpu.VMEM((NT, D + SPARE, LANES), F32),
            pltpu.VMEM((NT, LANES, LANES), F32),
            pltpu.VMEM((NT * NV, DH * 8, LANES), F32),
            pltpu.VMEM((KV, S), F32),
            pltpu.VMEM((NT + 1, D + 8, LANES), F32),
            pltpu.VMEM((NT + 1, H, LANES), F32),
            pltpu.VMEM((NMXU + 1, LANES, LANES), F32),
            pltpu.VMEM((GU_OFF[-1], LANES // 2, LANES), U32),
            pltpu.VMEM((NU, GU_OFF[-1], 2, LANES, LANES), BF16),
            pltpu.VMEM((NU, 49, QD, LANES), BF16),
            pltpu.VMEM((NU, 49, LANES, LANES), BF16),
            *[pltpu.VMEM((252 * 16 + SPARE, LANES), F32)] * 3,
            pltpu.SMEM((1,), jnp.int32),
            pltpu.SemaphoreType.DMA((12 + NB,)),
            pltpu.SemaphoreType.DMA((4 * NB,)),
        ],
        compiler_params=pltpu.CompilerParams(vmem_limit_bytes=120 * 2 ** 20),
        name="adaln_mqa_swiglu",
    )(c, A_wk.T, A_wv.T, A_x.reshape(S, D).T, A_wq, A_wo, B_w_gate, B_w_up, B_w_down.T, w_mod)
    return outT.T.reshape(1, S, D)
```
